```python
import os as _os
_os.environ.setdefault("JAX_PLATFORMS", "cpu")
import jax
import jax.numpy as jnp

def _softmax(x, axis=-1):
    return jax.nn.softmax(x, axis=axis)
def _gelu(x):
    return jax.nn.gelu(x, approximate=True)
def _silu(x):
    return jax.nn.silu(x)
def _sigmoid(x):
    return jax.nn.sigmoid(x)
def _layernorm(x, axis=-1, eps=1e-5):
    m = jnp.mean(x, axis=axis, keepdims=True)
    v = jnp.var(x, axis=axis, keepdims=True)
    return (x - m) / jnp.sqrt(v + eps)
def _scatter_add(tgt, idx, src, axis=0):
    return tgt.at[idx].add(src)
def _segment_sum(src, seg, n):
    return jax.ops.segment_sum(src, seg, n)
class _Rng:
    def __init__(self, key):
        self._k = key
    def _next(self):
        self._k, sub = jax.random.split(self._k)
        return sub
    def normal(self, shape):
        return jax.random.normal(self._next(), shape, dtype=jnp.bfloat16)
    def randint(self, lo, hi, shape):
        return jax.random.randint(self._next(), shape, lo, hi, dtype=jnp.int32)
    def uniform(self, shape, lo=0.0, hi=1.0):
        return jax.random.uniform(self._next(), shape, jnp.bfloat16, lo, hi)
    def permutation(self, n):
        return jax.random.permutation(self._next(), n)


kernel_name = 'concat_heads__gqa_block_cached__mha_block_cached__near_ridge'

def setup_inputs():
    _rng = _Rng(jax.random.key(int.from_bytes(__import__("os").urandom(4), "little")))
    _w = (lambda a: (lambda t: t.astype(jnp.bfloat16) if jnp.issubdtype(t.dtype, jnp.floating) else t)(jnp.asarray(a)))
    def _A_setup():
        B, Sq, D = 8, 112, 448
        Hq, Hkv, Sk, Dh = 16, 8, 512, 256
        assert Hq % Hkv == 0, (Hq, Hkv)
        return {
            "x": _w((lambda *s: _rng.normal(s) * 0.8)(B, Sq, D)),
            "k_cache": _w((lambda *s: _rng.normal(s) * 0.8)(B, Hkv, Sk, Dh)),
            "v_cache": _w((lambda *s: _rng.normal(s) * 0.05)(B, Hkv, Sk, Dh)),
            "wq": _w((lambda *s: _rng.normal(s) * 0.8)(D, Hq * Dh) * (D ** -0.5)),
            "wo": _w((lambda *s: _rng.normal(s) * 0.05)(Hq * Dh, D) * ((Hq * Dh) ** -0.5)),
        }
    _A_in = _A_setup()

    def _B_setup():
        B, Sq, D = 8, 112, 448
        H, Sk, Dh = 16, 512, 256
        return {
            "x": _w((lambda *s: _rng.normal(s) * 0.8)(B, Sq, D)),
            "k_cache": _w((lambda *s: _rng.normal(s) * 0.8)(B, H, Sk, Dh)),
            "v_cache": _w((lambda *s: _rng.normal(s) * 0.05)(B, H, Sk, Dh)),
            "wq": _w((lambda *s: _rng.normal(s) * 0.8)(D, H * Dh) * (D ** -0.5)),
            "wo": _w((lambda *s: _rng.normal(s) * 0.05)(H * Dh, D) * ((H * Dh) ** -0.5)),
        }
    _B_in = _B_setup()

    return {
        "A_x": _A_in["x"],
        "A_k_cache": _A_in["k_cache"],
        "A_v_cache": _A_in["v_cache"],
        "A_wq": _A_in["wq"],
        "A_wo": _A_in["wo"],
        "B_x": _B_in["x"],
        "B_k_cache": _B_in["k_cache"],
        "B_v_cache": _B_in["v_cache"],
        "B_wq": _B_in["wq"],
        "B_wo": _B_in["wo"],
    }

def reference(A_x, A_k_cache, A_v_cache, A_wq, A_wo, B_x, B_k_cache, B_v_cache, B_wq, B_wo):
    def _A_ref(x, k_cache, v_cache, wq, wo):
        B, Sq, D = x.shape
        Hq, Dh = 16, 256
        Hkv = k_cache.shape[1]
        rep = Hq // Hkv
        q = (lambda x, *d: x.transpose(*d))((x @ wq).reshape(B, Sq, Hq, Dh), 0, 2, 1, 3)
        k = jnp.repeat(k_cache, rep, axis=1)
        v = jnp.repeat(v_cache, rep, axis=1)
        scores = jnp.einsum("bhqd,bhkd->bhqk", q, k) * (Dh ** -0.5)
        p = _softmax(scores, axis=-1)
        o = jnp.einsum("bhqk,bhkd->bhqd", p, v)
        return (lambda x, *d: x.transpose(*d))(o, 0, 2, 1, 3).reshape(B, Sq, Hq * Dh) @ wo

    def _B_ref(x, k_cache, v_cache, wq, wo):
        B, Sq, D = x.shape
        H, Dh = 16, 256
        q = (lambda x, *d: x.transpose(*d))((x @ wq).reshape(B, Sq, H, Dh), 0, 2, 1, 3)
        scores = jnp.einsum("bhqd,bhkd->bhqk", q, k_cache) * (Dh ** -0.5)
        p = _softmax(scores, axis=-1)
        o = jnp.einsum("bhqk,bhkd->bhqd", p, v_cache)
        return (lambda x, *d: x.transpose(*d))(o, 0, 2, 1, 3).reshape(B, Sq, H * Dh) @ wo

    a = _A_ref(A_x, A_k_cache, A_v_cache, A_wq, A_wo)
    b = _B_ref(B_x, B_k_cache, B_v_cache, B_wq, B_wo)
    return jnp.concatenate([a, b], axis=-1)
```

```python
import jax
import jax.numpy as jnp
import numpy as np
import jax.experimental.pallas as pl
import jax.experimental.pallas.tpu as pltpu

B, SQ, D, SK, DH = 8, 112, 448, 512, 256
M = B * SQ
NP = 8
LAST = 2 * NP - 1
W = 2 * DH
NS = 16
NT_TILES = M // 128
QU = 2
QSCALE = float(DH ** -0.5 * np.log2(np.e))
NT = (((1,), (1,)), ((), ()))
F32, BF16 = jnp.float32, jnp.bfloat16
S_X, S_WQ, S_PAIR, S_FIN, S_OUT, S_N = 0, 2, 18, 48, 58, 60


def _kernel(xa_h, ka_h, va_h, wqa_h, woa_h, xb_h, kb_h, vb_h, wqb_h, wob_h, out_h,
            x_v, wq_v, wo_v, kv_v, q_v, o_v, acc_v, out_v, sem):
    def cp(src, dst, s):
        return pltpu.make_async_copy(src, dst, sem.at[s])

    def w_slice(refs, i):
        return refs[i // NP].at[:, pl.ds((i % NP) * W, W)]

    def wo_cp(i, s):
        return cp(w_slice((woa_h, wob_h), i), wo_v.at[i], s)

    def kslot(i):
        return i if i < NP else (2 * i - NP) % NS

    halves = (pl.ds(0, B // 2), pl.ds(B // 2, B // 2))

    def start_pairs(lo, hi):
        for i in range(lo, hi):
            parts = halves if i == LAST - 1 else (pl.ds(0, B),)
            for n, bs in enumerate(parts):
                s, k = S_PAIR + 2 * i + n, kslot(i)
                if i < NP:
                    cp(ka_h.at[bs, i], kv_v.at[k, bs, 0], s).start()
                    cp(va_h.at[bs, i], kv_v.at[k, bs, 1], s).start()
                else:
                    hs = pl.ds(2 * (i - NP), 2)
                    cp(kb_h.at[bs, hs], kv_v.at[k, bs], s).start()
                    cp(vb_h.at[bs, hs], kv_v.at[k + 1, bs], s).start()
            wo_cp(i, s).start()

    kl = kslot(LAST)

    def fin_cps(b):
        hs = pl.ds(2 * (LAST - NP), 2)
        sv = S_FIN + (B + 1 if b == B - 1 else b)
        return (cp(kb_h.at[b, hs], kv_v.at[kl, b], S_FIN + b),
                cp(vb_h.at[b, hs], kv_v.at[kl + 1, b], sv))

    for br, (x_h, wq_h) in enumerate(((xa_h, wqa_h), (xb_h, wqb_h))):
        cp(x_h, x_v.at[br], S_X + br).start()
        for i in range(br * NP, (br + 1) * NP):
            cp(w_slice((wqa_h, wqb_h), i), wq_v.at[i], S_WQ + i).start()
    start_pairs(0, NP)
    acc_v[...] = jnp.zeros_like(acc_v)

    def q_step(t, carry):
        br = t // (NP // QU)

        @pl.when(t % (NP // QU) == 0)
        def _():
            cp(xa_h, x_v.at[br], S_X + br).wait()

        for u in range(QU):
            i = t * QU + u
            cp(wqa_h.at[:, pl.ds(0, W)], wq_v.at[i], S_WQ + i).wait()
        for u in range(QU):
            i = t * QU + u
            q = jnp.dot(x_v[br], wq_v[i], preferred_element_type=F32)
            q_v[i] = (q * QSCALE).astype(BF16)
        return carry

    jax.lax.fori_loop(0, 2 * NP // QU, q_step, None)
    start_pairs(NP, NP + 4)

    def rows(b):
        return slice(b * SQ, (b + 1) * SQ)

    def cols(n):
        return slice(n * 128, (n + 1) * 128)

    def qk(i, b, j, k):
        s = jax.lax.dot_general(q_v[i, rows(b), j * DH:(j + 1) * DH], k, NT,
                                preferred_element_type=F32)
        p = jnp.exp2(s - jnp.max(s, axis=-1, keepdims=True))
        l = jnp.sum(p, axis=-1, keepdims=True)
        r = pl.reciprocal(l, approx=True)
        r = r * (2.0 - l * r)
        return p.astype(BF16), r

    def pv(b, j, v_idx, p, r):
        o = jnp.dot(p, kv_v[v_idx], preferred_element_type=F32)
        o_v[rows(b), j * DH:(j + 1) * DH] = (o * r).astype(BF16)

    def out_proj(i, n):
        return jax.lax.dot_general(wo_v[i], o_v[cols(n), :], NT, preferred_element_type=F32)

    def pair_compute(i, br, ks, acc_rows, before_second_half=None):
        pending = None
        for b in range(B):
            if b == B // 2 and before_second_half is not None:
                before_second_half()
            for j in range(2):
                item = (b, j, (ks + br, b, 1 if j else 1 - br)) + qk(i, b, j, kv_v[ks, b, j * br])
                if pending is not None:
                    pv(*pending)
                pending = item
        pv(*pending)
        for n in range(NT_TILES):
            acc_v[acc_rows, cols(n)] += out_proj(i, n)

    def wait_kv(slot, bs, s):
        cp(kb_h.at[bs, pl.ds(0, 2)], kv_v.at[slot, bs], s).wait()

    def wait_wo(i, s):
        cp(woa_h.at[:, pl.ds(0, W)], wo_v.at[i], s).wait()

    def pair_step(i, carry):
        br = i // NP
        ks = jnp.where(br == 0, i, (2 * i - NP) % NS)

        @pl.when(i == NP)
        def _():
            start_pairs(NP + 4, LAST)
            for b in range(B):
                for c in fin_cps(b):
                    c.start()
                if b == 1:
                    wo_cp(LAST, S_FIN + B).start()

        s = S_PAIR + 2 * i
        wait_kv(ks, pl.ds(0, B), s)

        @pl.when(br == 1)
        def _():
            wait_kv(ks + 1, pl.ds(0, B), s)

        wait_wo(i, s)
        pair_compute(i, br, ks, pl.ds(pl.multiple_of(br * D, 64), D))
        return carry

    jax.lax.fori_loop(0, LAST - 1, pair_step, None)

    i, ks = LAST - 1, kslot(LAST - 1)
    s = S_PAIR + 2 * i
    wait_kv(ks, halves[0], s)
    wait_kv(ks + 1, halves[0], s)

    def wait_second_half():
        wait_kv(ks, halves[1], s + 1)
        wait_kv(ks + 1, halves[1], s + 1)
        wait_wo(i, s + 1)

    pair_compute(i, 1, ks, pl.ds(D, D), wait_second_half)

    def finish(n):
        fb = acc_v[D:2 * D, cols(n)] + out_proj(LAST, n)
        out_v[cols(n), :] = jnp.concatenate([acc_v[0:D, cols(n)], fb], axis=0).T.astype(BF16)

    for b in range(B - 1):
        for c in fin_cps(b):
            c.wait()
        if b == 2:
            wo_cp(LAST, S_FIN + B).wait()
        a0 = qk(LAST, b, 0, kv_v[kl, b, 0])
        a1 = qk(LAST, b, 1, kv_v[kl, b, 1])
        if b >= 2:
            finish(b - 2)
        pv(b, 0, (kl + 1, b, 0), *a0)
        pv(b, 1, (kl + 1, b, 1), *a1)
    finish(NT_TILES - 2)

    b = B - 1
    head = pl.ds(0, M - 128)
    tail = pl.ds(M - 128, 128)
    ck, cv = fin_cps(b)
    ck.wait()
    a0 = qk(LAST, b, 0, kv_v[kl, b, 0])
    a1 = qk(LAST, b, 1, kv_v[kl, b, 1])
    cp(out_v.at[head], out_h.at[head], S_OUT).start()
    cv.wait()
    pv(b, 0, (kl + 1, b, 0), *a0)
    pv(b, 1, (kl + 1, b, 1), *a1)
    finish(NT_TILES - 1)
    cp(out_v.at[tail], out_h.at[tail], S_OUT + 1).start()
    cp(out_v.at[head], out_h.at[head], S_OUT).wait()
    cp(out_v.at[tail], out_h.at[tail], S_OUT + 1).wait()


@jax.jit
def pallas_concat_heads__gqa_block_cached__mha_block_cached__near_ridge_kernel(
    A_x: jax.Array,
    A_k_cache: jax.Array,
    A_v_cache: jax.Array,
    A_wq: jax.Array,
    A_wo: jax.Array,
    B_x: jax.Array,
    B_k_cache: jax.Array,
    B_v_cache: jax.Array,
    B_wq: jax.Array,
    B_wo: jax.Array,
):
    hbm = pl.BlockSpec(memory_space=pltpu.HBM)
    out = pl.pallas_call(
        _kernel,
        in_specs=[hbm] * 10,
        out_specs=hbm,
        out_shape=jax.ShapeDtypeStruct((M, 2 * D), BF16),
        scratch_shapes=[
            pltpu.VMEM((2, M, D), BF16),
            pltpu.VMEM((2 * NP, D, W), BF16),
            pltpu.VMEM((2 * NP, D, W), BF16),
            pltpu.VMEM((NS, B, 2, SK, DH), BF16),
            pltpu.VMEM((2 * NP, M, W), BF16),
            pltpu.VMEM((M, W), BF16),
            pltpu.VMEM((2 * D, M), F32),
            pltpu.VMEM((M, 2 * D), BF16),
            pltpu.SemaphoreType.DMA((S_N,)),
        ],
        compiler_params=pltpu.CompilerParams(
            vmem_limit_bytes=120 << 20,
            disable_bounds_checks=True,
            flags={"XLA_TPU_RESCHEDULE_DMA_DONES": True},
        ),
    )(A_x.reshape(M, D), A_k_cache, A_v_cache, A_wq, A_wo.T,
      B_x.reshape(M, D), B_k_cache, B_v_cache, B_wq, B_wo.T)
    return out.reshape(B, SQ, 2 * D)
```

```python
import jax
import jax.numpy as jnp
import numpy as np
import jax.experimental.pallas as pl
import jax.experimental.pallas.tpu as pltpu

B, SQ, D, SK, DH = 8, 112, 448, 512, 256
M = B * SQ
NP = 8
LAST = 2 * NP - 1
W = 2 * DH
NS = 16
TILE = 128
CUTS = (0, 4, 6, 8)
QSCALE = float(DH ** -0.5 * np.log2(np.e))
NT = (((1,), (1,)), ((), ()))
F32, BF16 = jnp.float32, jnp.bfloat16

TAIL = (
    ("wait", ("k", 0), ("k", 1), ("v", 0)), ("qk", 0), ("qk", 1), ("pv", 0),
    ("wait", ("k", 2), ("v", 1), ("wo", 0)), ("qk", 2), ("pv", 1),
    ("wait", ("k", 3), ("v", 2)), ("qk", 3), ("out", 0), ("pv", 2),
    ("wait", ("k", 4), ("v", 3)), ("qk", 4), ("out", 1), ("pv", 3),
    ("wait", ("k", 5), ("v", 4)), ("pv", 4), ("out", 2), ("qk", 5), ("out", 3),
    ("wait", ("k", 6), ("v", 5)), ("pv", 5), ("qk", 6), ("out", 4),
    ("wait", ("k", 7)), ("qk", 7),
    ("wait", ("v", 6)), ("write", 0, 5), ("pv", 6),
    ("wait", ("v", 7)), ("pv", 7), ("out", 5), ("out", 6), ("write", 5, 7),
)
S_Q, S_WO, S_PAIR, S_TAIL = 0, 5, 7, 24
S_N = S_TAIL + len(TAIL)


def _softmax_parts(s):
    p = jnp.exp2(s - jnp.max(s, axis=-1, keepdims=True))
    l = jnp.sum(p, axis=-1, keepdims=True)
    r = pl.reciprocal(l, approx=True)
    r = r * (2.0 - l * r)
    return p.astype(BF16), r


def _kernel(xa_h, ka_h, va_h, wqa_h, woa_h, xb_h, kb_h, vb_h, wqb_h, wob_h, out_h,
            x_v, wq_v, wo_v, kv_v, q_v, o_v, acc_v, out_v, sem):
    def cp(src, dst, s):
        return pltpu.make_async_copy(src, dst, sem.at[s])

    def start(copies):
        for c in copies:
            c.start()

    def wait(copies):
        for c in copies:
            c.wait()

    def wcols(i):
        g = i % NP
        return pl.ds(g * W if isinstance(g, int) else pl.multiple_of(g * W, W), W)

    def rows(b):
        return pl.ds(b * SQ, SQ)

    def tile(n):
        return pl.ds(n * TILE, TILE)

    half = M // 2

    def xa_cp(n):
        r = pl.ds(n * half, half)
        return cp(xa_h.at[r], x_v.at[0, r], S_Q + n)

    def wqa_cp(lo, hi, s):
        c = pl.ds(lo * W, (hi - lo) * W)
        return cp(wqa_h.at[:, c], wq_v.at[0, :, c], s)

    def wo_cp(br, lo, hi, s):
        c = pl.ds(lo * W, (hi - lo) * W)
        return cp((woa_h, wob_h)[br].at[:, c], wo_v.at[br, :, c], s)

    def kslot(i):
        return i if i < NP else (2 * i - NP) % NS

    def pair_cps(i, lo, hi, s):
        bs, k = pl.ds(lo, hi - lo), kslot(i)
        if i < NP:
            return [cp(ka_h.at[bs, i], kv_v.at[k, bs, 0], s),
                    cp(va_h.at[bs, i], kv_v.at[k, bs, 1], s)]
        hs = pl.ds(2 * (i - NP), 2)
        return [cp(kb_h.at[bs, hs], kv_v.at[k, bs], s),
                cp(vb_h.at[bs, hs], kv_v.at[k + 1, bs], s)]

    def prelast_cps(n):
        s = S_PAIR + LAST - 1 + n
        copies = pair_cps(LAST - 1, CUTS[n], CUTS[n + 1], s)
        if n == len(CUTS) - 2:
            copies.append(wo_cp(1, NP - 2, NP - 1, s))
        return copies

    kl = kslot(LAST)

    def tail_cps(step):
        hs, s = pl.ds(2 * (NP - 1), 2), S_TAIL + step
        copies = []
        for kind, b in TAIL[step][1:]:
            if kind == "k":
                copies.append(cp(kb_h.at[b, hs], kv_v.at[kl, b], s))
            elif kind == "v":
                copies.append(cp(vb_h.at[b, hs], kv_v.at[kl + 1, b], s))
            else:
                copies.append(wo_cp(1, NP - 1, NP, s))
        return copies

    q_cps = ([wqa_cp(0, 1, S_Q), xa_cp(0)],
             [xa_cp(1)],
             [wqa_cp(1, 4, S_Q + 2)],
             [wqa_cp(4, NP, S_Q + 3)],
             [cp(xb_h, x_v.at[1], S_Q + 4), cp(wqb_h, wq_v.at[1], S_Q + 4)])
    for copies in q_cps:
        start(copies)
    wo_cp(0, 0, NP, S_WO).start()
    for i in range(NP):
        start(pair_cps(i, 0, B, S_PAIR + i))
    acc_v[...] = jnp.zeros_like(acc_v)

    def q_proj(i, r):
        q = jnp.dot(x_v[i // NP, r], wq_v[i // NP, :, wcols(i)], preferred_element_type=F32)
        q_v[i, r] = (q * QSCALE).astype(BF16)

    for n in range(2):
        wait(q_cps[n])
        q_proj(0, pl.ds(n * half, half))

    def q_step(t, carry):
        for at in range(3):
            @pl.when(t == at)
            def _():
                wait(q_cps[2 + at])

        for u in range(3):
            q_proj(1 + 3 * t + u, pl.ds(0, M))
        return carry

    jax.lax.fori_loop(0, LAST // 3, q_step, None)

    wo_cp(1, 0, NP - 2, S_WO + 1).start()
    for i in range(NP, NP + 4):
        start(pair_cps(i, 0, B, S_PAIR + i))

    def out_proj(br, i, n):
        return jax.lax.dot_general(wo_v[br, :, wcols(i)], o_v[tile(n), :], NT,
                                   preferred_element_type=F32)

    def accumulate(br, i):
        for n in range(M // TILE):
            acc_v[br * D:(br + 1) * D, tile(n)] += out_proj(br, i, n)

    def wait_slot(slot, s):
        cp(kb_h.at[:, pl.ds(0, 2)], kv_v.at[slot], s).wait()

    def gqa_step(i, carry):
        wait_slot(i, S_PAIR + i)

        def pv(b, p, r):
            o = (jnp.dot(p, kv_v[i, b, 1], preferred_element_type=F32) * r).astype(BF16)
            o_v[rows(b), 0:DH] = o[:SQ]
            o_v[rows(b), DH:W] = o[SQ:]

        pending = None
        for b in range(B):
            q = jnp.concatenate([q_v[i, rows(b), 0:DH], q_v[i, rows(b), DH:W]], axis=0)
            s = jax.lax.dot_general(q, kv_v[i, b, 0], NT, preferred_element_type=F32)
            item = (b,) + _softmax_parts(s)
            if pending is not None:
                pv(*pending)
            pending = item
        pv(*pending)
        accumulate(0, i)
        return carry

    wo_cp(0, 0, NP, S_WO).wait()
    jax.lax.fori_loop(0, NP, gqa_step, None)

    for i in range(NP + 4, LAST - 1):
        start(pair_cps(i, 0, B, S_PAIR + i))
    for n in range(len(CUTS) - 1):
        start(prelast_cps(n))
    for step, op in enumerate(TAIL):
        if op[0] == "wait":
            start(tail_cps(step))

    def mha_qk(i, ks, b, j):
        q = q_v[i, rows(b), j * DH:(j + 1) * DH]
        return _softmax_parts(
            jax.lax.dot_general(q, kv_v[ks, b, j], NT, preferred_element_type=F32))

    def mha_pv(ks, b, j, p, r):
        o = jnp.dot(p, kv_v[ks + 1, b, j], preferred_element_type=F32)
        o_v[rows(b), j * DH:(j + 1) * DH] = (o * r).astype(BF16)

    def mha_pair(i, ks, before_batch=None):
        pending = None
        for b in range(B):
            if before_batch is not None:
                before_batch(b)
            for j in range(2):
                item = (ks, b, j) + mha_qk(i, ks, b, j)
                if pending is not None:
                    mha_pv(*pending)
                pending = item
        mha_pv(*pending)
        accumulate(1, i)

    def mha_step(i, carry):
        ks = (2 * i - NP) % NS
        wait_slot(ks, S_PAIR + i)
        wait_slot(ks + 1, S_PAIR + i)
        mha_pair(i, ks)
        return carry

    wo_cp(1, 0, NP - 2, S_WO + 1).wait()
    jax.lax.fori_loop(NP, LAST - 1, mha_step, None)

    def prelast_wait(b):
        if b in CUTS:
            wait(prelast_cps(CUTS.index(b)))

    mha_pair(LAST - 1, kslot(LAST - 1), prelast_wait)

    probs, writes = {}, []
    for step, op in enumerate(TAIL):
        if op[0] == "wait":
            wait(tail_cps(step))
        elif op[0] == "qk":
            probs[op[1]] = [mha_qk(LAST, kl, op[1], j) for j in range(2)]
        elif op[0] == "pv":
            for j in range(2):
                mha_pv(kl, op[1], j, *probs[op[1]][j])
        elif op[0] == "out":
            t = tile(op[1])
            out_b = acc_v[D:2 * D, t] + out_proj(1, LAST, op[1])
            out_v[t, :] = jnp.concatenate([acc_v[0:D, t], out_b], axis=0).T.astype(BF16)
        else:
            r = pl.ds(op[1] * TILE, (op[2] - op[1]) * TILE)
            writes.append(cp(out_v.at[r], out_h.at[r], S_TAIL + step))
            writes[-1].start()
    wait(writes)


@jax.jit
def pallas_concat_heads__gqa_block_cached__mha_block_cached__near_ridge_kernel(
    A_x: jax.Array,
    A_k_cache: jax.Array,
    A_v_cache: jax.Array,
    A_wq: jax.Array,
    A_wo: jax.Array,
    B_x: jax.Array,
    B_k_cache: jax.Array,
    B_v_cache: jax.Array,
    B_wq: jax.Array,
    B_wo: jax.Array,
):
    hbm = pl.BlockSpec(memory_space=pltpu.HBM)
    out = pl.pallas_call(
        _kernel,
        in_specs=[hbm] * 10,
        out_specs=hbm,
        out_shape=jax.ShapeDtypeStruct((M, 2 * D), BF16),
        scratch_shapes=[
            pltpu.VMEM((2, M, D), BF16),
            pltpu.VMEM((2, D, NP * W), BF16),
            pltpu.VMEM((2, D, NP * W), BF16),
            pltpu.VMEM((NS, B, 2, SK, DH), BF16),
            pltpu.VMEM((2 * NP, M, W), BF16),
            pltpu.VMEM((M, W), BF16),
            pltpu.VMEM((2 * D, M), F32),
            pltpu.VMEM((M, 2 * D), BF16),
            pltpu.SemaphoreType.DMA((S_N,)),
        ],
        compiler_params=pltpu.CompilerParams(vmem_limit_bytes=120 << 20),
    )(A_x.reshape(M, D), A_k_cache, A_v_cache, A_wq, A_wo.T,
      B_x.reshape(M, D), B_k_cache, B_v_cache, B_wq, B_wo.T)
    return out.reshape(B, SQ, 2 * D)
```

```python
import jax
import jax.numpy as jnp
import numpy as np
import jax.experimental.pallas as pl
import jax.experimental.pallas.tpu as pltpu

B, SQ, D, SK, DH = 8, 112, 448, 512, 256
M = B * SQ
NP = 8
LAST = 2 * NP - 1
W = 2 * DH
NS = 16
TILE = 128
CUTS = (0, 4, 6, 8)
QSCALE = float(DH ** -0.5 * np.log2(np.e))
NT = (((1,), (1,)), ((), ()))
F32, BF16 = jnp.float32, jnp.bfloat16

TAIL = (
    ("wait", ("k", 0), ("k", 1), ("v", 0)), ("qk", 0), ("qk", 1), ("pv", 0),
    ("wait", ("k", 2), ("v", 1), ("wo", 0)), ("qk", 2), ("pv", 1),
    ("wait", ("k", 3), ("v", 2)), ("qk", 3), ("out", 0), ("pv", 2),
    ("wait", ("k", 4), ("v", 3)), ("qk", 4), ("out", 1), ("pv", 3),
    ("wait", ("k", 5), ("v", 4)), ("pv", 4), ("out", 2), ("qk", 5), ("out", 3),
    ("wait", ("k", 6), ("v", 5)), ("pv", 5), ("qk", 6), ("out", 4),
    ("wait", ("k", 7)), ("qk", 7),
    ("wait", ("v", 6)), ("write", 0, 5), ("pv", 6),
    ("wait", ("v", 7)), ("pv", 7), ("out", 5), ("out", 6), ("write", 5, 7),
)
NSEM = 4


def _softmax_parts(s):
    p = jnp.exp2(s - jnp.max(s, axis=-1, keepdims=True))
    l = jnp.sum(p, axis=-1, keepdims=True)
    r = pl.reciprocal(l, approx=True)
    r = r * (2.0 - l * r)
    return p.astype(BF16), r


def _kernel(xa_h, ka_h, va_h, wqa_h, woa_h, xb_h, kb_h, vb_h, wqb_h, wob_h, out_h,
            x_v, wq_v, wo_v, kv_v, q_v, o_v, acc_v, out_v, sem):
    def wcols(i):
        g = i % NP
        return pl.ds(g * W if isinstance(g, int) else pl.multiple_of(g * W, W), W)

    def rows(b):
        return pl.ds(b * SQ, SQ)

    def tile(n):
        return pl.ds(n * TILE, TILE)

    half = M // 2

    def xa_part(n):
        r = pl.ds(n * half, half)
        return [(xa_h.at[r], x_v.at[0, r])]

    def w_part(w_h, w_v, br, lo, hi):
        c = pl.ds(lo * W, (hi - lo) * W)
        return [(w_h.at[:, c], w_v.at[br, :, c])]

    def kslot(i):
        return i if i < NP else (2 * i - NP) % NS

    def kv_part(pairs, lo=0, hi=B):
        bs, parts = pl.ds(lo, hi - lo), []
        for i in pairs:
            k = kslot(i)
            if i < NP:
                parts += [(ka_h.at[bs, i], kv_v.at[k, bs, 0]), (va_h.at[bs, i], kv_v.at[k, bs, 1])]
            else:
                hs = pl.ds(2 * (i - NP), 2)
                parts += [(kb_h.at[bs, hs], kv_v.at[k, bs]), (vb_h.at[bs, hs], kv_v.at[k + 1, bs])]
        return parts

    kl = kslot(LAST)

    def tail_part(kind, b):
        hs = pl.ds(2 * (NP - 1), 2)
        if kind == "k":
            return (kb_h.at[b, hs], kv_v.at[kl, b])
        if kind == "v":
            return (vb_h.at[b, hs], kv_v.at[kl + 1, b])
        return w_part(wob_h, wo_v, 1, NP - 1, NP)[0]

    groups = [
        w_part(wqa_h, wq_v, 0, 0, 1) + xa_part(0),
        xa_part(1),
        w_part(wqa_h, wq_v, 0, 1, 4),
        w_part(wqa_h, wq_v, 0, 4, NP),
        [(xb_h, x_v.at[1]), (wqb_h, wq_v.at[1])],
        [(woa_h, wo_v.at[0])] + kv_part(range(0, 4)),
        kv_part(range(4, 8)),
        w_part(wob_h, wo_v, 1, 0, NP - 2) + kv_part((8, 9)),
        kv_part((10, 11)),
        kv_part((12,)),
        kv_part((13,)),
        kv_part((14,), CUTS[0], CUTS[1]),
        kv_part((14,), CUTS[1], CUTS[2]),
        kv_part((14,), CUTS[2], CUTS[3]) + w_part(wob_h, wo_v, 1, NP - 2, NP - 1),
    ]
    n_loads = len(groups) + sum(op[0] == "wait" for op in TAIL)
    groups += [[tail_part(*part) for part in op[1:]] for op in TAIL if op[0] == "wait"]
    for op in TAIL:
        if op[0] == "write":
            r = pl.ds(op[1] * TILE, (op[2] - op[1]) * TILE)
            groups.append([(out_v.at[r], out_h.at[r])])

    def start(n):
        for src, dst in groups[n]:
            pltpu.make_async_copy(src, dst, sem.at[n % NSEM]).start()

    def wait(n, refill=True):
        for src, dst in groups[n]:
            pltpu.make_async_copy(src, dst, sem.at[n % NSEM]).wait()
        if refill and n + NSEM < n_loads:
            start(n + NSEM)

    def wait_at(index, plan, refill=True):
        for at, n in plan:
            @pl.when(index == at)
            def _():
                wait(n, refill)

    for n in range(NSEM):
        start(n)
    acc_v[...] = jnp.zeros_like(acc_v)

    def q_proj(i, r):
        q = jnp.dot(x_v[i // NP, r], wq_v[i // NP, :, wcols(i)], preferred_element_type=F32)
        q_v[i, r] = (q * QSCALE).astype(BF16)

    for n in range(2):
        wait(n)
        q_proj(0, pl.ds(n * half, half))

    def q_step(t, carry):
        wait_at(t, ((0, 2), (1, 3), (2, 4)))
        for u in range(3):
            q_proj(1 + 3 * t + u, pl.ds(0, M))
        return carry

    jax.lax.fori_loop(0, LAST // 3, q_step, None)

    def out_proj(br, i, n):
        return jax.lax.dot_general(wo_v[br, :, wcols(i)], o_v[tile(n), :], NT,
                                   preferred_element_type=F32)

    def accumulate(br, i):
        for n in range(M // TILE):
            acc_v[br * D:(br + 1) * D, tile(n)] += out_proj(br, i, n)

    def gqa_step(i, carry):
        wait_at(i, ((4, 6),), refill=False)

        def pv(b, p, r):
            o = (jnp.dot(p, kv_v[i, b, 1], preferred_element_type=F32) * r).astype(BF16)
            o_v[rows(b), 0:DH] = o[:SQ]
            o_v[rows(b), DH:W] = o[SQ:]

        pending = None
        for b in range(B):
            q = jnp.concatenate([q_v[i, rows(b), 0:DH], q_v[i, rows(b), DH:W]], axis=0)
            s = jax.lax.dot_general(q, kv_v[i, b, 0], NT, preferred_element_type=F32)
            item = (b,) + _softmax_parts(s)
            if pending is not None:
                pv(*pending)
            pending = item
        pv(*pending)
        accumulate(0, i)
        return carry

    wait(5, refill=False)
    jax.lax.fori_loop(0, NP, gqa_step, None)

    start(5 + NSEM)
    start(6 + NSEM)

    def mha_qk(i, ks, b, j):
        q = q_v[i, rows(b), j * DH:(j + 1) * DH]
        return _softmax_parts(
            jax.lax.dot_general(q, kv_v[ks, b, j], NT, preferred_element_type=F32))

    def mha_pv(ks, b, j, p, r):
        o = jnp.dot(p, kv_v[ks + 1, b, j], preferred_element_type=F32)
        o_v[rows(b), j * DH:(j + 1) * DH] = (o * r).astype(BF16)

    def mha_pair(i, ks, before_batch=None):
        pending = None
        for b in range(B):
            if before_batch is not None:
                before_batch(b)
            for j in range(2):
                item = (ks, b, j) + mha_qk(i, ks, b, j)
                if pending is not None:
                    mha_pv(*pending)
                pending = item
        mha_pv(*pending)
        accumulate(1, i)

    def mha_step(i, carry):
        wait_at(i, ((10, 8), (12, 9), (13, 10)))
        mha_pair(i, (2 * i - NP) % NS)
        return carry

    wait(7)
    jax.lax.fori_loop(NP, LAST - 1, mha_step, None)

    def prelast_wait(b):
        if b in CUTS:
            wait(11 + CUTS.index(b))

    mha_pair(LAST - 1, kslot(LAST - 1), prelast_wait)

    probs, load, write = {}, 14, n_loads
    for op in TAIL:
        if op[0] == "wait":
            wait(load)
            load += 1
        elif op[0] == "qk":
            probs[op[1]] = [mha_qk(LAST, kl, op[1], j) for j in range(2)]
        elif op[0] == "pv":
            for j in range(2):
                mha_pv(kl, op[1], j, *probs[op[1]][j])
        elif op[0] == "out":
            t = tile(op[1])
            out_b = acc_v[D:2 * D, t] + out_proj(1, LAST, op[1])
            out_v[t, :] = jnp.concatenate([acc_v[0:D, t], out_b], axis=0).T.astype(BF16)
        else:
            assert write - NSEM < load
            start(write)
            write += 1
    for n in range(n_loads, write):
        wait(n)


@jax.jit
def pallas_concat_heads__gqa_block_cached__mha_block_cached__near_ridge_kernel(
    A_x: jax.Array,
    A_k_cache: jax.Array,
    A_v_cache: jax.Array,
    A_wq: jax.Array,
    A_wo: jax.Array,
    B_x: jax.Array,
    B_k_cache: jax.Array,
    B_v_cache: jax.Array,
    B_wq: jax.Array,
    B_wo: jax.Array,
):
    hbm = pl.BlockSpec(memory_space=pltpu.HBM)
    out = pl.pallas_call(
        _kernel,
        in_specs=[hbm] * 10,
        out_specs=hbm,
        out_shape=jax.ShapeDtypeStruct((M, 2 * D), BF16),
        scratch_shapes=[
            pltpu.VMEM((2, M, D), BF16),
            pltpu.VMEM((2, D, NP * W), BF16),
            pltpu.VMEM((2, D, NP * W), BF16),
            pltpu.VMEM((NS, B, 2, SK, DH), BF16),
            pltpu.VMEM((2 * NP, M, W), BF16),
            pltpu.VMEM((M, W), BF16),
            pltpu.VMEM((2 * D, M), F32),
            pltpu.VMEM((M, 2 * D), BF16),
            pltpu.SemaphoreType.DMA((NSEM,)),
        ],
        compiler_params=pltpu.CompilerParams(vmem_limit_bytes=120 << 20),
    )(A_x.reshape(M, D), A_k_cache, A_v_cache, A_wq, A_wo.T,
      B_x.reshape(M, D), B_k_cache, B_v_cache, B_wq, B_wo.T)
    return out.reshape(B, SQ, 2 * D)
```
